```python
import jax
import jax.numpy as jnp

def _softmax(x, axis=-1):
    return jax.nn.softmax(x, axis=axis)
def _gelu(x):
    return jax.nn.gelu(x, approximate=True)
def _silu(x):
    return jax.nn.silu(x)
def _sigmoid(x):
    return jax.nn.sigmoid(x)
def _layernorm(x, axis=-1, eps=1e-5):
    m = jnp.mean(x, axis=axis, keepdims=True)
    v = jnp.var(x, axis=axis, keepdims=True)
    return (x - m) / jnp.sqrt(v + eps)
def _scatter_add(tgt, idx, src, axis=0):
    return tgt.at[idx].add(src)
def _segment_sum(src, seg, n):
    return jax.ops.segment_sum(src, seg, n)
class _Rng:
    def __init__(self, key):
        self._k = key
    def _next(self):
        self._k, sub = jax.random.split(self._k)
        return sub
    def normal(self, shape):
        return jax.random.normal(self._next(), shape, dtype=jnp.bfloat16)
    def randint(self, lo, hi, shape):
        return jax.random.randint(self._next(), shape, lo, hi, dtype=jnp.int32)
    def uniform(self, shape, lo=0.0, hi=1.0):
        return jax.random.uniform(self._next(), shape, jnp.bfloat16, lo, hi)
    def permutation(self, n):
        return jax.random.permutation(self._next(), n)


kernel_name = 'interleave_layers__sliding_local_dilated__glu_gated_bilinear__prompt'

def setup_inputs():
    _rng = _Rng(jax.random.key(int.from_bytes(__import__("os").urandom(4), "little")))
    _w = (lambda a: (lambda t: t.astype(jnp.bfloat16) if jnp.issubdtype(t.dtype, jnp.floating) else t)(jnp.asarray(a)))
    def _A_setup():
        B, S, D = 1, 2048, 576
        return {
            "x": _w((lambda *s: _rng.normal(s) * 0.05)(B, S, D)),
            "wqkv": _w((lambda *s: _rng.normal(s) * 0.05)(D, 3 * D)),
            "wo": _w((lambda *s: _rng.normal(s) * 0.05)(D, D)),
        }
    _A_in = _A_setup()

    def _B_setup():
        B, S, D, F = 1, 2048, 576, 4608
        return {
            "x": _w((lambda *s: _rng.normal(s) * 0.05)(B, S, D)),
            "w_gate": _w((lambda *s: _rng.normal(s) * 0.05)(D, F) * (D ** -0.5)),
            "w_up": _w((lambda *s: _rng.normal(s) * 0.05)(D, F) * (D ** -0.5)),
            "w_down": _w((lambda *s: _rng.normal(s) * 0.05)(F, D) * (F ** -0.5)),
        }
    _B_in = _B_setup()

    return {
        "A_x": _A_in["x"],
        "A_wqkv": _A_in["wqkv"],
        "A_wo": _A_in["wo"],
        "B_x": _B_in["x"],
        "B_w_gate": _B_in["w_gate"],
        "B_w_up": _B_in["w_up"],
        "B_w_down": _B_in["w_down"],
    }

def reference(A_x, A_wqkv, A_wo, B_x, B_w_gate, B_w_up, B_w_down):
    def _A_ref(x, wqkv, wo):
        B, S, D = x.shape
        H = 32; Dh = D // H
        W, dil = 8, 2
        qkv = (lambda x, *d: x.transpose(*d))((x @ wqkv).reshape(B, S, 3, H, Dh), 2, 0, 3, 1, 4)
        q, k, v = qkv[0], qkv[1], qkv[2]
        scale = Dh ** -0.5
        pos = jnp.arange(S)
        off = jnp.arange(W) * dil
        idx = pos[:, None] - off[None, :]
        mask = idx >= 0
        idx_c = jnp.where(mask, idx, 0).reshape(-1)
        kg = k[:, :, idx_c, :].reshape(B, H, S, W, Dh)
        vg = v[:, :, idx_c, :].reshape(B, H, S, W, Dh)
        logits = jnp.einsum("bhsd,bhswd->bhsw", q, kg) * scale
        logits = jnp.where(mask[None, None, :, :], logits, -1e9)
        attn = _softmax(logits, axis=-1)
        o = jnp.einsum("bhsw,bhswd->bhsd", attn, vg)
        return (lambda x, *d: x.transpose(*d))(o, 0, 2, 1, 3).reshape(B, S, D) @ wo

    def _B_ref(x, w_gate, w_up, w_down):
        g = jnp.einsum("bsd,df->bsf", x, w_gate)
        u = jnp.einsum("bsd,df->bsf", x, w_up)
        h = g * u
        return jnp.einsum("bsf,fd->bsd", h, w_down)

    x = A_x
    x = x + _A_ref(_layernorm(x, axis=-1), A_wqkv, A_wo)
    x = x + _B_ref(_layernorm(x, axis=-1), B_w_gate, B_w_up, B_w_down)
    x = x + _A_ref(_layernorm(x, axis=-1), A_wqkv, A_wo)
    x = x + _B_ref(_layernorm(x, axis=-1), B_w_gate, B_w_up, B_w_down)
    return x
```

```python
import jax
import jax.numpy as jnp
import jax.experimental.pallas as pl
import jax.experimental.pallas.tpu as pltpu

S, D, F, H, DH, W = 2048, 576, 4608, 32, 18, 8
NC = 8
NCHUNK = 4
FC = F // NCHUNK
FT = 384
bf16, f32, u32 = jnp.bfloat16, jnp.float32, jnp.uint32
NN = (((1,), (0,)), ((), ()))
NT = (((1,), (1,)), ((), ()))


def _dot(a, b, dn=NN):
    return jax.lax.dot_general(a, b, dn, preferred_element_type=f32)


def _tr(a):
    parts = [a[:, j * 128:(j + 1) * 128].T for j in range(4)]
    tail = jnp.concatenate([a[:, 512:], jnp.zeros((128, 64), a.dtype)], axis=1).T[:64]
    return jnp.concatenate(parts + [tail], axis=0)


def _tr_back(a):
    parts = [a[j * 128:(j + 1) * 128].T for j in range(4)]
    tail = jnp.concatenate([a[512:], jnp.zeros((64, 128), a.dtype)], axis=0).T[:, :64]
    return jnp.concatenate(parts + [tail], axis=1)


def _ln(x):
    m = jnp.mean(x, axis=0, keepdims=True)
    xc = x - m
    v = jnp.mean(xc * xc, axis=0, keepdims=True)
    return xc / jnp.sqrt(v + 1e-5)


def _kernel(x_hbm, wqkv_hbm, wo_hbm, wg_hbm, wu_hbm, wd_hbm, out_hbm,
            xin, wqkv, wo, wg, wu, wd, wtmp, wqkvT, woT, wdT,
            xT, xn, q, kx, vx, oT, hbuf, sems):
    cp = lambda src, dst, i: pltpu.make_async_copy(src, dst, sems.at[i])
    c_x, c_qkv, c_o = cp(x_hbm, xin, 0), cp(wqkv_hbm, wqkv, 1), cp(wo_hbm, wo, 2)
    c_g, c_u, c_d = cp(wg_hbm, wg, 3), cp(wu_hbm, wu, 4), cp(wd_hbm, wd, 5)
    c_qkv.start()
    c_x.start()
    c_o.start()

    def put(r0, a):
        a = jnp.concatenate([a, jnp.zeros((a.shape[0], 64), a.dtype)], axis=1)
        for k in range(5):
            wtmp[pl.ds(k * 3 * D + r0, a.shape[0]), :] = a[:, k * 128:(k + 1) * 128]

    def get(r0, n, stride):
        return jnp.concatenate(
            [wtmp[pl.ds(k * 3 * D + r0, n, stride=stride), :] for k in range(5)], axis=1)[:, :D]

    c_qkv.wait()
    for j in range(14):
        n = min(128, 3 * D - j * 128)
        blk = wqkv[:, j * 128:j * 128 + n].astype(f32)
        if n < 128:
            blk = jnp.concatenate([blk, jnp.zeros((D, 128 - n), f32)], axis=1)
        put(j * 128, _tr_back(blk)[:n])
    for t in range(3):
        for d in range(DH):
            wqkvT[pl.ds(t * D + d * H, H), :] = get(t * D + d, H, DH).astype(bf16)

    c_x.wait()
    c_d.start()
    c_g.start()
    c_u.start()
    xw = xin.bitcast(u32)
    for r in range(NC):
        put(r * 128, pltpu.bitcast(xw[r * 128:(r + 1) * 128, :], f32))
    for r in range(NC):
        wds = pltpu.bitcast(_tr(get(r, 128, NC)), u32)
        xT[0, r] = pltpu.bitcast(wds << 16, f32)
        xT[1, r] = pltpu.bitcast(wds & jnp.uint32(0xFFFF0000), f32)

    lane0 = jax.lax.broadcasted_iota(jnp.int32, (8, 128), 1) == 0
    scale = DH ** -0.5

    def qkv_proj(s):
        for r in range(0, NC, 2):
            xb = jnp.concatenate([_ln(xT[s, r]).astype(bf16), _ln(xT[s, r + 1]).astype(bf16)], axis=1)
            y = _dot(wqkvT[...], xb)
            for i in range(2):
                c = r + i
                yy = y[:, i * 128:(i + 1) * 128]
                q[c] = yy[:D] * scale
                kx[c + 7] = yy[D:2 * D]
                vx[c + 7] = yy[2 * D:]
                if c >= 1:
                    kx[c - 1] = pltpu.roll(yy[D:2 * D], 1, 1)
                    vx[c - 1] = jnp.where(
                        jax.lax.broadcasted_iota(jnp.int32, (D, 128), 1) == 0,
                        0.0, pltpu.roll(yy[2 * D:], 1, 1))

    def attn_piece(s, r, hg):
        rows = lambda d: pl.ds(pl.multiple_of(d * H + hg * 8, 8), 8)
        qs = [q[r, rows(d), :] for d in range(DH)]
        ls = []
        for w in range(W):
            c = r - w + 7
            acc = qs[0] * kx[c, rows(0), :]
            for d in range(1, DH):
                acc = acc + qs[d] * kx[c, rows(d), :]
            if w > r:
                acc = jnp.where(lane0, -1e9, acc)
            ls.append(acc)
        m = ls[0]
        for l in ls[1:]:
            m = jnp.maximum(m, l)
        es = [jnp.exp(l - m) for l in ls]
        den = es[0]
        for e in es[1:]:
            den = den + e
        inv = 1.0 / den
        ps = [e * inv for e in es]
        for d in range(DH):
            acc = ps[0] * vx[r + 7, rows(d), :]
            for w in range(1, W):
                acc = acc + ps[w] * vx[r - w + 7, rows(d), :]
            oT[s, rows(d), r * 128:(r + 1) * 128] = acc

    def attn_group(s, hg):
        for r in range(NC):
            attn_piece(s, r, hg)

    qkv_proj(0)
    c_o.wait()
    put(0, wo[...].astype(f32))
    for d in range(DH):
        put(D + d * H, get(d, H, DH))
    for j in range(5):
        n = min(128, D - j * 128)
        blk = get(D + j * 128, n, 1)
        if n < 128:
            blk = jnp.concatenate([blk, jnp.zeros((128 - n, D), f32)], axis=0)
        woT[:, j * 128:j * 128 + n] = _tr(blk)[:, :n].astype(bf16)

    def pro(hg, c):
        attn_group(0, hg)
        return c
    jax.lax.fori_loop(0, H // 8, pro, 0)

    c_d.wait()

    def wd_tr(j, c):
        o = pl.multiple_of(j * 128, 128)
        wdT[:, pl.ds(o, 128)] = _tr(wd[pl.ds(o, 128), :].astype(f32)).astype(bf16)
        return c
    jax.lax.fori_loop(0, F // 128, wd_tr, 0)
    c_g.wait()
    c_u.wait()

    def step(t, carry):
        s = t % 2
        o = 1 - s
        for r in range(0, NC, 2):
            y = _dot(woT[...], oT[s, :, r * 128:(r + 2) * 128].astype(bf16))
            for i in range(2):
                c = r + i
                x1 = xT[s, c] + y[:, i * 128:(i + 1) * 128]
                xT[s, c] = x1
                xn[c * 128:(c + 1) * 128, :] = _tr_back(_ln(x1)).astype(bf16)

        @pl.when(t < 3)
        def _():
            qkv_proj(o)

        def chunk(ci, c):
            f0 = pl.multiple_of(ci * FC, 128)
            for j in range(0, FC, FT):
                fs = pl.ds(pl.multiple_of(f0 + j, 128), FT)
                for mb in range(0, NC * 128, 512):
                    xa = xn[mb:mb + 512, :]
                    hbuf[mb:mb + 512, j:j + FT] = (_dot(xa, wg[:, fs]) * _dot(xa, wu[:, fs])).astype(bf16)
            for r in range(0, NC, 4):
                y = _dot(wdT[:, pl.ds(f0, FC)], hbuf[r * 128:(r + 4) * 128, :], NT)
                for i in range(4):
                    xT[s, r + i] += y[:, i * 128:(i + 1) * 128]
            attn_group(o, ci)
            return c
        jax.lax.fori_loop(0, NCHUNK, chunk, 0)
        return carry
    jax.lax.fori_loop(0, 4, step, 0)

    for r in range(NC):
        lo = pltpu.bitcast(xT[0, r].astype(bf16).astype(f32), u32) >> 16
        hi = pltpu.bitcast(xT[1, r].astype(bf16).astype(f32), u32)
        wds = pltpu.bitcast(lo | hi, f32)
        for k in range(5):
            blk = wds[k * 128:(k + 1) * 128]
            if k == 4:
                blk = jnp.concatenate([blk, jnp.zeros((64, 128), f32)], axis=0)
            wtmp[pl.ds(k * 3 * D + r, 128, stride=NC), :] = blk.T
    for r in range(NC):
        xw[r * 128:(r + 1) * 128, :] = pltpu.bitcast(get(r * 128, 128, 1), u32)
    c_out = cp(xin, out_hbm, 6)
    c_out.start()
    c_out.wait()


@jax.jit
def pallas_interleave_layers__sliding_local_dilated__glu_gated_bilinear__prompt_kernel(
    A_x: jax.Array,
    A_wqkv: jax.Array,
    A_wo: jax.Array,
    B_x: jax.Array,
    B_w_gate: jax.Array,
    B_w_up: jax.Array,
    B_w_down: jax.Array,
):
    del B_x
    V = pltpu.VMEM
    out = pl.pallas_call(
        _kernel,
        out_shape=jax.ShapeDtypeStruct((S, D), bf16),
        in_specs=[pl.BlockSpec(memory_space=pl.ANY)] * 6,
        out_specs=pl.BlockSpec(memory_space=pl.ANY),
        scratch_shapes=[
            V((S, D), bf16), V((D, 3 * D), bf16), V((D, D), bf16),
            V((D, F), bf16), V((D, F), bf16), V((F, D), bf16),
            V((5 * 3 * D, 128), f32), V((3 * D, D), bf16), V((D, D), bf16), V((D, F), bf16),
            V((2, NC, D, 128), f32), V((NC * 128, D), bf16),
            V((NC, D, 128), f32), V((2 * NC - 1, D, 128), f32), V((2 * NC - 1, D, 128), f32),
            V((2, D, NC * 128), f32), V((NC * 128, FC), bf16),
            pltpu.SemaphoreType.DMA((7,)),
        ],
        compiler_params=pltpu.CompilerParams(vmem_limit_bytes=110 * 2**20),
    )(A_x.reshape(S, D), A_wqkv, A_wo, B_w_gate, B_w_up, B_w_down)
    return out.reshape(1, S, D)
```

```python
import jax
import jax.numpy as jnp
import jax.experimental.pallas as pl
import jax.experimental.pallas.tpu as pltpu

S, D, F, H, DH, W = 2048, 576, 4608, 32, 18, 8
NC = 8
NCHUNK = 4
FC = F // NCHUNK
FT = 384
bf16, f32, u32 = jnp.bfloat16, jnp.float32, jnp.uint32
NN = (((1,), (0,)), ((), ()))
NT = (((1,), (1,)), ((), ()))


def _dot(a, b, dn=NN):
    return jax.lax.dot_general(a, b, dn, preferred_element_type=f32)


def _tr(a):
    parts = [a[:, j * 128:(j + 1) * 128].T for j in range(4)]
    tail = jnp.concatenate([a[:, 512:], jnp.zeros((128, 64), a.dtype)], axis=1).T[:64]
    return jnp.concatenate(parts + [tail], axis=0)


def _tr_back(a):
    parts = [a[j * 128:(j + 1) * 128].T for j in range(4)]
    tail = jnp.concatenate([a[512:], jnp.zeros((64, 128), a.dtype)], axis=0).T[:, :64]
    return jnp.concatenate(parts + [tail], axis=1)


def _ln(x):
    m = jnp.mean(x, axis=0, keepdims=True)
    xc = x - m
    v = jnp.mean(xc * xc, axis=0, keepdims=True)
    return xc / jnp.sqrt(v + 1e-5)


def _kernel(x_hbm, wqkv_hbm, wo_hbm, wg_hbm, wu_hbm, wd_hbm, out_hbm,
            xin, wqkv, wo, wg, wu, xs, wtmp, wqkvT, woT, wdT,
            xT, xn, q, kx, vx, oT, hbuf, sems):
    cp = lambda src, dst, i: pltpu.make_async_copy(src, dst, sems.at[i])
    c_x, c_qkv, c_o = cp(x_hbm, xin, 0), cp(wqkv_hbm, wqkv, 1), cp(wo_hbm, wo, 2)
    c_g, c_u, c_d = cp(wg_hbm, wg, 3), cp(wu_hbm, wu, 4), cp(wd_hbm, wdT, 5)
    c_qkv.start()
    c_x.start()
    c_o.start()

    def put(r0, a):
        a = jnp.concatenate([a, jnp.zeros((a.shape[0], 64), a.dtype)], axis=1)
        for k in range(5):
            wtmp[pl.ds(k * 3 * D + r0, a.shape[0]), :] = a[:, k * 128:(k + 1) * 128]

    def get(r0, n, stride):
        return jnp.concatenate(
            [wtmp[pl.ds(k * 3 * D + r0, n, stride=stride), :] for k in range(5)], axis=1)[:, :D]

    c_qkv.wait()
    for j in range(14):
        n = min(128, 3 * D - j * 128)
        blk = wqkv[:, j * 128:j * 128 + n].astype(f32)
        if n < 128:
            blk = jnp.concatenate([blk, jnp.zeros((D, 128 - n), f32)], axis=1)
        put(j * 128, _tr_back(blk)[:n])
    for t in range(3):
        for d in range(DH):
            wqkvT[pl.ds(t * D + d * H, H), :] = get(t * D + d, H, DH).astype(bf16)

    c_x.wait()
    c_d.start()
    c_g.start()
    c_u.start()
    xw = xin.bitcast(u32)
    z32 = jnp.zeros((96, 128), f32)
    for c in range(2 * NC):
        a = jnp.concatenate([pltpu.bitcast(xw[:, c * 128:(c + 1) * 128], f32), z32], axis=0)
        for k in range(3):
            xs[pl.ds(k * S + c * 128, 128), :] = a[k * 128:(k + 1) * 128].T
    for c in range(2 * NC):
        a = jnp.concatenate(
            [xs[pl.ds(k * S + c, 128, stride=2 * NC), :].T for k in range(3)], axis=0)[:D // 2]
        xT[c % 2, c // 2] = pltpu.bitcast(a, bf16).astype(f32)

    lane0 = jax.lax.broadcasted_iota(jnp.int32, (8, 128), 1) == 0
    scale = DH ** -0.5

    def qkv_proj(s):
        for r in range(0, NC, 2):
            xb = jnp.concatenate([_ln(xT[s, r]).astype(bf16), _ln(xT[s, r + 1]).astype(bf16)], axis=1)
            y = _dot(wqkvT[...], xb)
            for i in range(2):
                c = r + i
                yy = y[:, i * 128:(i + 1) * 128]
                q[c] = yy[:D] * scale
                kx[c + 7] = yy[D:2 * D]
                vx[c + 7] = yy[2 * D:]
                if c >= 1:
                    kx[c - 1] = pltpu.roll(yy[D:2 * D], 1, 1)
                    vx[c - 1] = jnp.where(
                        jax.lax.broadcasted_iota(jnp.int32, (D, 128), 1) == 0,
                        0.0, pltpu.roll(yy[2 * D:], 1, 1))

    def attn_piece(s, r, hg):
        rows = lambda d: pl.ds(pl.multiple_of(d * H + hg * 8, 8), 8)
        qs = [q[r, rows(d), :] for d in range(DH)]
        ls = []
        for w in range(W):
            c = r - w + 7
            acc = qs[0] * kx[c, rows(0), :]
            for d in range(1, DH):
                acc = acc + qs[d] * kx[c, rows(d), :]
            if w > r:
                acc = jnp.where(lane0, -1e9, acc)
            ls.append(acc)
        m = ls[0]
        for l in ls[1:]:
            m = jnp.maximum(m, l)
        es = [jnp.exp(l - m) for l in ls]
        den = es[0]
        for e in es[1:]:
            den = den + e
        inv = 1.0 / den
        ps = [e * inv for e in es]
        for d in range(DH):
            acc = ps[0] * vx[r + 7, rows(d), :]
            for w in range(1, W):
                acc = acc + ps[w] * vx[r - w + 7, rows(d), :]
            oT[s, rows(d), r * 128:(r + 1) * 128] = acc

    def attn_group(s, hg):
        for r in range(NC):
            attn_piece(s, r, hg)

    qkv_proj(0)
    c_o.wait()
    put(0, wo[...].astype(f32))
    for d in range(DH):
        put(D + d * H, get(d, H, DH))
    for j in range(5):
        n = min(128, D - j * 128)
        blk = get(D + j * 128, n, 1)
        if n < 128:
            blk = jnp.concatenate([blk, jnp.zeros((128 - n, D), f32)], axis=0)
        woT[:, j * 128:j * 128 + n] = _tr(blk)[:, :n].astype(bf16)

    def pro(hg, c):
        attn_group(0, hg)
        return c
    jax.lax.fori_loop(0, H // 8, pro, 0)

    c_d.wait()
    c_g.wait()
    c_u.wait()

    def step(t, carry):
        s = t % 2
        o = 1 - s
        for r in range(0, NC, 2):
            y = _dot(woT[...], oT[s, :, r * 128:(r + 2) * 128].astype(bf16))
            for i in range(2):
                c = r + i
                x1 = xT[s, c] + y[:, i * 128:(i + 1) * 128]
                xT[s, c] = x1
                xn[c * 128:(c + 1) * 128, :] = _tr_back(_ln(x1)).astype(bf16)

        @pl.when(t < 3)
        def _():
            qkv_proj(o)

        def chunk(ci, c):
            f0 = pl.multiple_of(ci * FC, 128)
            for j in range(0, FC, FT):
                fs = pl.ds(pl.multiple_of(f0 + j, 128), FT)
                for mb in range(0, NC * 128, 512):
                    xa = xn[mb:mb + 512, :]
                    hbuf[mb:mb + 512, j:j + FT] = (_dot(xa, wg[:, fs]) * _dot(xa, wu[:, fs])).astype(bf16)
            for r in range(0, NC, 4):
                y = _dot(wdT[:, pl.ds(f0, FC)], hbuf[r * 128:(r + 4) * 128, :], NT)
                for i in range(4):
                    xT[s, r + i] += y[:, i * 128:(i + 1) * 128]
            attn_group(o, ci)
            return c
        jax.lax.fori_loop(0, NCHUNK, chunk, 0)
        return carry
    jax.lax.fori_loop(0, 4, step, 0)

    for c in range(2 * NC):
        a = jnp.concatenate([pltpu.bitcast(xT[c % 2, c // 2].astype(bf16), f32), z32], axis=0)
        for k in range(3):
            xs[pl.ds(k * S + c, 128, stride=2 * NC), :] = a[k * 128:(k + 1) * 128].T
    for c in range(2 * NC):
        a = jnp.concatenate(
            [xs[pl.ds(k * S + c * 128, 128), :].T for k in range(3)], axis=0)[:D // 2]
        xw[:, c * 128:(c + 1) * 128] = pltpu.bitcast(a, u32)
    c_out = cp(xin, out_hbm, 6)
    c_out.start()
    c_out.wait()


@jax.jit
def pallas_interleave_layers__sliding_local_dilated__glu_gated_bilinear__prompt_kernel(
    A_x: jax.Array,
    A_wqkv: jax.Array,
    A_wo: jax.Array,
    B_x: jax.Array,
    B_w_gate: jax.Array,
    B_w_up: jax.Array,
    B_w_down: jax.Array,
):
    del B_x
    V = pltpu.VMEM
    out = pl.pallas_call(
        _kernel,
        out_shape=jax.ShapeDtypeStruct((D, S), bf16),
        in_specs=[pl.BlockSpec(memory_space=pltpu.MemorySpace.HBM)] * 6,
        out_specs=pl.BlockSpec(memory_space=pltpu.MemorySpace.HBM),
        scratch_shapes=[
            V((D, S), bf16), V((D, 3 * D), bf16), V((D, D), bf16),
            V((D, F), bf16), V((D, F), bf16), V((3 * S, 128), f32),
            V((5 * 3 * D, 128), f32), V((3 * D, D), bf16), V((D, D), bf16), V((D, F), bf16),
            V((2, NC, D, 128), f32), V((NC * 128, D), bf16),
            V((NC, D, 128), f32), V((2 * NC - 1, D, 128), f32), V((2 * NC - 1, D, 128), f32),
            V((2, D, NC * 128), f32), V((NC * 128, FC), bf16),
            pltpu.SemaphoreType.DMA((7,)),
        ],
        compiler_params=pltpu.CompilerParams(vmem_limit_bytes=110 * 2**20),
    )(A_x[0].T, A_wqkv, A_wo, B_w_gate, B_w_up, B_w_down.T)
    return out.T[None]
```

```python
import jax
import jax.numpy as jnp
import jax.experimental.pallas as pl
import jax.experimental.pallas.tpu as pltpu

S, D, F, H, DH, W = 2048, 576, 4608, 32, 18, 8
NC = 8
NCHUNK = 9
FC = F // NCHUNK
FT = 512
bf16, f32, u32 = jnp.bfloat16, jnp.float32, jnp.uint32
NN = (((1,), (0,)), ((), ()))
NT = (((1,), (1,)), ((), ()))


def _dot(a, b, dn=NN):
    return jax.lax.dot_general(a, b, dn, preferred_element_type=f32)


def _tr(a):
    parts = [a[:, j * 128:(j + 1) * 128].T for j in range(4)]
    tail = jnp.concatenate([a[:, 512:], jnp.zeros((128, 64), a.dtype)], axis=1).T[:64]
    return jnp.concatenate(parts + [tail], axis=0)


def _tr_back(a):
    parts = [a[j * 128:(j + 1) * 128].T for j in range(4)]
    tail = jnp.concatenate([a[512:], jnp.zeros((64, 128), a.dtype)], axis=0).T[:, :64]
    return jnp.concatenate(parts + [tail], axis=1)


def _ln(x):
    m = jnp.mean(x, axis=0, keepdims=True)
    xc = x - m
    v = jnp.mean(xc * xc, axis=0, keepdims=True)
    return xc * (1.0 / jnp.sqrt(v + 1e-5))


def _kernel(x_hbm, wqkv_hbm, wo_hbm, wg_hbm, wu_hbm, wd_hbm, out_hbm,
            xin, wqkv, wo, wg, wu, xs, wtmp, wqkvT, woT, wdT,
            xT, xn, q, kx, vx, oT, hbuf, sems):
    cp = lambda src, dst, i: pltpu.make_async_copy(src, dst, sems.at[i])
    c_x, c_qkv, c_o = cp(x_hbm, xin, 0), cp(wqkv_hbm, wqkv, 1), cp(wo_hbm, wo, 2)
    c_g, c_u, c_d = cp(wg_hbm, wg, 3), cp(wu_hbm, wu, 4), cp(wd_hbm, wdT, 5)
    c_qkv.start()
    c_x.start()
    c_o.start()

    def put(r0, a):
        a = jnp.concatenate([a, jnp.zeros((a.shape[0], 64), a.dtype)], axis=1)
        for k in range(5):
            wtmp[pl.ds(k * 3 * D + r0, a.shape[0]), :] = a[:, k * 128:(k + 1) * 128]

    def get(r0, n, stride):
        return jnp.concatenate(
            [wtmp[pl.ds(k * 3 * D + r0, n, stride=stride), :] for k in range(5)], axis=1)[:, :D]

    c_qkv.wait()
    for j in range(14):
        n = min(128, 3 * D - j * 128)
        blk = wqkv[:, j * 128:j * 128 + n].astype(f32)
        if n < 128:
            blk = jnp.concatenate([blk, jnp.zeros((D, 128 - n), f32)], axis=1)
        put(j * 128, _tr_back(blk)[:n])
    for t in range(3):
        for d in range(DH):
            wqkvT[pl.ds(t * D + d * H, H), :] = get(t * D + d, H, DH).astype(bf16)

    c_x.wait()
    c_d.start()
    c_g.start()
    c_u.start()
    xw = xin.bitcast(u32)
    z32 = jnp.zeros((96, 128), f32)
    for c in range(2 * NC):
        a = jnp.concatenate([pltpu.bitcast(xw[:, c * 128:(c + 1) * 128], f32), z32], axis=0)
        for k in range(3):
            xs[pl.ds(k * S + c * 128, 128), :] = a[k * 128:(k + 1) * 128].T
    for c in range(2 * NC):
        a = jnp.concatenate(
            [xs[pl.ds(k * S + c, 128, stride=2 * NC), :].T for k in range(3)], axis=0)[:D // 2]
        xT[c % 2, c // 2] = pltpu.bitcast(a, bf16).astype(f32)

    lane = jax.lax.broadcasted_iota(jnp.int32, (8, 128), 1)
    scale = DH ** -0.5

    def qkv_proj(s):
        for r in range(0, NC, 4):
            xb = jnp.concatenate([_ln(xT[s, r + i]).astype(bf16) for i in range(4)], axis=1)
            y = _dot(wqkvT[...], xb)
            for i in range(4):
                c = r + i
                yy = y[:, i * 128:(i + 1) * 128]
                q[c] = yy[:D] * scale
                kx[c + 7] = yy[D:2 * D]
                vx[c + 7] = yy[2 * D:]
                if c >= 1:
                    kx[c - 1] = pltpu.roll(yy[D:2 * D], 1, 1)
                    vx[c - 1] = jnp.where(
                        jax.lax.broadcasted_iota(jnp.int32, (D, 128), 1) == 0,
                        0.0, pltpu.roll(yy[2 * D:], 1, 1))

    def attn_piece(s, r, hg):
        rows = lambda d: pl.ds(d * H + hg * 8, 8)
        qs = [q[r, rows(d), :] for d in range(DH)]
        ls = []
        for w in range(W):
            c = r - w + 7
            acc = qs[0] * kx[c, rows(0), :]
            for d in range(1, DH):
                acc = acc + qs[d] * kx[c, rows(d), :]
            if w:
                acc = jnp.where(lane < jnp.where(w > r, 1, 0), -1e9, acc)
            ls.append(acc)
        m = ls[0]
        for l in ls[1:]:
            m = jnp.maximum(m, l)
        es = [jnp.exp(l - m) for l in ls]
        den = es[0]
        for e in es[1:]:
            den = den + e
        inv = 1.0 / den
        ps = [e * inv for e in es]
        for d in range(DH):
            acc = ps[0] * vx[r + 7, rows(d), :]
            for w in range(1, W):
                acc = acc + ps[w] * vx[r - w + 7, rows(d), :]
            oT[s, r, rows(d), :] = acc

    def attn_group(s, r):
        for hg in range(H // 8):
            attn_piece(s, r, hg)

    qkv_proj(0)
    c_o.wait()
    put(0, wo[...].astype(f32))
    for d in range(DH):
        put(D + d * H, get(d, H, DH))
    for j in range(5):
        n = min(128, D - j * 128)
        blk = get(D + j * 128, n, 1)
        if n < 128:
            blk = jnp.concatenate([blk, jnp.zeros((128 - n, D), f32)], axis=0)
        woT[:, j * 128:j * 128 + n] = _tr(blk)[:, :n].astype(bf16)

    def pro(hg, c):
        attn_group(0, hg)
        return c
    jax.lax.fori_loop(0, NC, pro, 0)

    c_d.wait()
    c_g.wait()
    c_u.wait()

    def step(t, carry):
        s = t % 2
        o = 1 - s
        for r in range(0, NC, 4):
            y = _dot(woT[...], jnp.concatenate([oT[s, r + i].astype(bf16) for i in range(4)], axis=1))
            for i in range(4):
                c = r + i
                x1 = xT[s, c] + y[:, i * 128:(i + 1) * 128]
                xT[s, c] = x1
                xn[c * 128:(c + 1) * 128, :] = _tr_back(_ln(x1)).astype(bf16)

        @pl.when(t < 3)
        def _():
            qkv_proj(o)

            def att(r, c):
                attn_group(o, r)
                return c
            jax.lax.fori_loop(0, NC, att, 0)

        def chunk(ci, c):
            f0 = pl.multiple_of(ci * FC, 128)
            for j in range(0, FC, FT):
                fs = pl.ds(pl.multiple_of(f0 + j, 128), FT)
                for mb in range(0, NC * 128, 1024):
                    xa = xn[mb:mb + 1024, :]
                    hbuf[mb:mb + 1024, j:j + FT] = (_dot(xa, wg[:, fs]) * _dot(xa, wu[:, fs])).astype(bf16)
            for r in range(0, NC, 4):
                y = _dot(wdT[:, pl.ds(f0, FC)], hbuf[r * 128:(r + 4) * 128, :], NT)
                for i in range(4):
                    xT[s, r + i] += y[:, i * 128:(i + 1) * 128]
            return c
        jax.lax.fori_loop(0, NCHUNK, chunk, 0)
        return carry
    jax.lax.fori_loop(0, 4, step, 0)

    for c in range(2 * NC):
        a = jnp.concatenate([pltpu.bitcast(xT[c % 2, c // 2].astype(bf16), f32), z32], axis=0)
        for k in range(3):
            xs[pl.ds(k * S + c, 128, stride=2 * NC), :] = a[k * 128:(k + 1) * 128].T
    for c in range(2 * NC):
        a = jnp.concatenate(
            [xs[pl.ds(k * S + c * 128, 128), :].T for k in range(3)], axis=0)[:D // 2]
        xw[:, c * 128:(c + 1) * 128] = pltpu.bitcast(a, u32)
    c_out = cp(xin, out_hbm, 6)
    c_out.start()
    c_out.wait()


@jax.jit
def pallas_interleave_layers__sliding_local_dilated__glu_gated_bilinear__prompt_kernel(
    A_x: jax.Array,
    A_wqkv: jax.Array,
    A_wo: jax.Array,
    B_x: jax.Array,
    B_w_gate: jax.Array,
    B_w_up: jax.Array,
    B_w_down: jax.Array,
):
    del B_x
    V = pltpu.VMEM
    out = pl.pallas_call(
        _kernel,
        out_shape=jax.ShapeDtypeStruct((D, S), bf16),
        in_specs=[pl.BlockSpec(memory_space=pltpu.MemorySpace.HBM)] * 6,
        out_specs=pl.BlockSpec(memory_space=pltpu.MemorySpace.HBM),
        scratch_shapes=[
            V((D, S), bf16), V((D, 3 * D), bf16), V((D, D), bf16),
            V((D, F), bf16), V((D, F), bf16), V((3 * S, 128), f32),
            V((5 * 3 * D, 128), f32), V((3 * D, D), bf16), V((D, D), bf16), V((D, F), bf16),
            V((2, NC, D, 128), f32), V((NC * 128, D), bf16),
            V((NC, D, 128), f32), V((2 * NC - 1, D, 128), f32), V((2 * NC - 1, D, 128), f32),
            V((2, NC, D, 128), f32), V((NC * 128, FC), bf16),
            pltpu.SemaphoreType.DMA((7,)),
        ],
        compiler_params=pltpu.CompilerParams(vmem_limit_bytes=110 * 2**20, flags={'XLA_TPU_EVENLY_DISTRIBUTE_CRITICAL_NODES':True}),
    )(A_x[0].T, A_wqkv, A_wo, B_w_gate, B_w_up, B_w_down.T)
    return out.T[None]
```
